```python
import os as _os
_os.environ.setdefault("JAX_PLATFORMS", "cpu")
import jax
import jax.numpy as jnp

def _softmax(x, axis=-1):
    return jax.nn.softmax(x, axis=axis)
def _gelu(x):
    return jax.nn.gelu(x, approximate=True)
def _silu(x):
    return jax.nn.silu(x)
def _sigmoid(x):
    return jax.nn.sigmoid(x)
def _layernorm(x, axis=-1, eps=1e-5):
    m = jnp.mean(x, axis=axis, keepdims=True)
    v = jnp.var(x, axis=axis, keepdims=True)
    return (x - m) / jnp.sqrt(v + eps)
def _scatter_add(tgt, idx, src, axis=0):
    return tgt.at[idx].add(src)
def _segment_sum(src, seg, n):
    return jax.ops.segment_sum(src, seg, n)
class _Rng:
    def __init__(self, key):
        self._k = key
    def _next(self):
        self._k, sub = jax.random.split(self._k)
        return sub
    def normal(self, shape):
        return jax.random.normal(self._next(), shape, dtype=jnp.bfloat16)
    def randint(self, lo, hi, shape):
        return jax.random.randint(self._next(), shape, lo, hi, dtype=jnp.int32)
    def uniform(self, shape, lo=0.0, hi=1.0):
        return jax.random.uniform(self._next(), shape, jnp.bfloat16, lo, hi)
    def permutation(self, n):
        return jax.random.permutation(self._next(), n)


kernel_name = 'concat_heads__sliding_block__sliding_block__prompt'

def setup_inputs():
    _rng = _Rng(jax.random.key(int.from_bytes(__import__("os").urandom(4), "little")))
    _w = (lambda a: (lambda t: t.astype(jnp.bfloat16) if jnp.issubdtype(t.dtype, jnp.floating) else t)(jnp.asarray(a)))
    def _A_setup():
        B, S, D = 1, 2048, 448
        return {
            "x": _w((lambda *s: _rng.normal(s) * 0.2)(B, S, D)),
            "wqkv": _w((lambda *s: _rng.normal(s) * 0.2)(D, 3 * D)),
            "wo": _w((lambda *s: _rng.normal(s) * 0.05)(D, D)),
        }
    _A_in = _A_setup()

    def _B_setup():
        B, S, D = 1, 2048, 448
        return {
            "x": _w((lambda *s: _rng.normal(s) * 0.2)(B, S, D)),
            "wqkv": _w((lambda *s: _rng.normal(s) * 0.2)(D, 3 * D)),
            "wo": _w((lambda *s: _rng.normal(s) * 0.05)(D, D)),
        }
    _B_in = _B_setup()

    return {
        "A_x": _A_in["x"],
        "A_wqkv": _A_in["wqkv"],
        "A_wo": _A_in["wo"],
        "B_x": _B_in["x"],
        "B_wqkv": _B_in["wqkv"],
        "B_wo": _B_in["wo"],
    }

def reference(A_x, A_wqkv, A_wo, B_x, B_wqkv, B_wo):
    def _A_ref(x, wqkv, wo):
        B, S, D = x.shape
        H = 16; Dh = D // H; W = 256
        qkv = (lambda x, *d: x.transpose(*d))((x @ wqkv).reshape(B, S, 3, H, Dh), 2, 0, 3, 1, 4)
        q, k, v = qkv[0], qkv[1], qkv[2]
        scores = jnp.einsum("bhqd,bhkd->bhqk", q, k) * (Dh ** -0.5)
        idx = jnp.arange(S)
        mask = (idx[:, None] - idx[None, :] >= 0) & (idx[:, None] - idx[None, :] < W)
        scores = jnp.where(mask[None, None], scores, -1e9)
        p = _softmax(scores, axis=-1)
        o = jnp.einsum("bhqk,bhkd->bhqd", p, v)
        return (lambda x, *d: x.transpose(*d))(o, 0, 2, 1, 3).reshape(B, S, D) @ wo

    def _B_ref(x, wqkv, wo):
        B, S, D = x.shape
        H = 16; Dh = D // H; W = 256
        qkv = (lambda x, *d: x.transpose(*d))((x @ wqkv).reshape(B, S, 3, H, Dh), 2, 0, 3, 1, 4)
        q, k, v = qkv[0], qkv[1], qkv[2]
        scores = jnp.einsum("bhqd,bhkd->bhqk", q, k) * (Dh ** -0.5)
        idx = jnp.arange(S)
        mask = (idx[:, None] - idx[None, :] >= 0) & (idx[:, None] - idx[None, :] < W)
        scores = jnp.where(mask[None, None], scores, -1e9)
        p = _softmax(scores, axis=-1)
        o = jnp.einsum("bhqk,bhkd->bhqd", p, v)
        return (lambda x, *d: x.transpose(*d))(o, 0, 2, 1, 3).reshape(B, S, D) @ wo

    a = _A_ref(A_x, A_wqkv, A_wo)
    b = _B_ref(B_x, B_wqkv, B_wo)
    return jnp.concatenate([a, b], axis=-1)
```

```python
import functools
import math

import jax
import jax.numpy as jnp
import jax.experimental.pallas as pl
import jax.experimental.pallas.tpu as pltpu

S = 2048
D = 448
H = 16
DH = 28
WIN = 256
T = 256
QB = 128
NQ = T // QB
KR = WIN + 32
HIST = WIN - 96
NSB = 12
LAG = 1
ORDER = "a"
NEG = -1e30
F32 = jnp.float32
BF16 = jnp.bfloat16
U32 = jnp.uint32
NT = (((1,), (1,)), ((), ()))
TN = (((0,), (0,)), ((), ()))


def _pack(x):
    return pltpu.bitcast(x.astype(BF16), U32)


def _unpack(x):
    return pltpu.bitcast(x, BF16)


def _kernel(xa_ref, wa_ref, woa_ref, xb_ref, wb_ref, wob_ref, o_ref,
            wvt_ref, wot_ref, ks_ref, vkh_ref, vt_ref, ot_ref, s_ref):
    i = pl.program_id(0)
    x_refs = (xa_ref, xb_ref)
    w_refs = (wa_ref, wb_ref)
    wo_refs = (woa_ref, wob_ref)

    def prep():
        z4 = jnp.zeros((4, D), F32)
        for br in range(2):
            wvt = w_refs[br][:, 2 * D:3 * D].T.astype(F32)
            for h in range(H):
                wvt_ref[br, 32 * h:32 * h + 32, :] = jnp.concatenate(
                    [wvt[DH * h:DH * h + DH], z4], axis=0).astype(BF16)
            wo = wo_refs[br][...].astype(F32)
            wop = jnp.concatenate(
                [jnp.concatenate([wo[DH * h:DH * h + DH], z4], axis=0) for h in range(H)], axis=0)
            wot_ref[br] = wop.astype(BF16).T
            ks_ref[br, :, 0:HIST // 2, :] = jnp.zeros((H, HIST // 2, 128), U32)
            vkh_ref[br] = jnp.zeros((4, 48, 128), U32)
            vt_ref[br, 0:2] = jnp.zeros((2, 256, 128), U32)

    def body(first):
        c = (DH ** -0.5) * math.log2(math.e)
        lane = jax.lax.broadcasted_iota(jnp.int32, (1, 128), 1)
        if first:
            row0 = 0
            tile0 = 0
        else:
            row0 = pl.multiple_of(i * (T // 2), T // 2)
            tile0 = i * NQ

        jj = jax.lax.broadcasted_iota(jnp.int32, (32, 128), 0)
        ql = jax.lax.broadcasted_iota(jnp.int32, (32, 128), 1) % 32
        diag_ok = jj <= ql
        j2 = 2 * jax.lax.broadcasted_iota(jnp.int32, (16, 128), 0)
        q2 = jax.lax.broadcasted_iota(jnp.int32, (16, 128), 1) % 32
        dmask = (jnp.where(j2 <= q2, jnp.uint32(0xFFFF), jnp.uint32(0))
                 | jnp.where(j2 + 1 <= q2, jnp.uint32(0xFFFF0000), jnp.uint32(0)))
        fmask = ~dmask
        m5 = (lane & 32) != 0
        m6 = (lane & 64) != 0

        st = {"x": {}, "tiles": {}, "rq": {}, "m": {}, "unit": 0, "sb": {}, "ot": {}}

        def proj_qk(br, t):
            if br not in st["x"]:
                st["x"][br] = x_refs[br][...].T
            tl = jnp.dot(st["x"][br], w_refs[br][:, 128 * t:128 * t + 128], preferred_element_type=F32)
            if t < 3:
                tl = tl * c
            elif t == 3:
                tl = tl * jnp.where(lane < 64, c, 1.0)
            st["tiles"][br, t] = _pack(tl)

        def proj_v(br, t):
            vt = jnp.dot(wvt_ref[br], x_refs[br][:, 128 * t:128 * t + 128], preferred_element_type=F32)
            rr = jax.lax.broadcasted_iota(jnp.int32, (512, 128), 0) % 32
            vt = jnp.where(rr == DH, 1.0, vt)
            vt_ref[br, tile0 + 2 + t] = _pack(vt)

        def build(br, a):
            tiles = lambda t: st["tiles"][br, t]
            cq = 112 * a
            tq, pq = cq // 128, cq % 128
            vq = tiles(tq) if pq + 112 <= 128 else jnp.where(lane >= pq, tiles(tq), tiles(tq + 1))
            ck = D + 112 * a
            tk, pk = ck // 128, ck % 128
            vk = tiles(tk) if pk + 112 <= 128 else jnp.where(lane >= pk, tiles(tk), tiles(tk + 1))
            chunks = []
            for ch in range(T // 32):
                g = ch % 4
                sh = (pk - pq + 32 * g) % 128
                blk = vq[16 * ch:16 * ch + 16]
                chunks.append(blk if sh == 0 else pltpu.roll(blk, sh, 1))
            st["rq"][br, a] = chunks
            vkx = jnp.concatenate([vkh_ref[br, a], vk], axis=0)
            vkh_ref[br, a] = vk[T // 2 - 48:]
            z = []
            for g in range(4):
                blk = vkx[16 * g:16 * g + T // 2]
                z.append(blk if g == 0 else pltpu.roll(blk, 32 * g, 1))
            for b in range(4):
                lp = (lane - (pk + DH * b)) & 127
                k5 = (lp & 32) != 0
                k6 = (lp & 64) != 0
                ksk = jnp.where(k6, jnp.where(k5, z[3], z[2]), jnp.where(k5, z[1], z[0]))
                ks_ref[br, 4 * a + b, pl.ds(row0 + HIST // 2, T // 2), :] = ksk

        def scores(br, qb, h):
            a, b = h // 4, h % 4
            pk = (D + 112 * a) % 128
            lp = (lane - (pk + DH * b)) & 127
            wt = []
            for g in range(4):
                msk = (lp >= 32 * g) & (lp < 32 * g + DH)
                wt.append(jnp.where(msk, st["rq"][br, a][4 * qb + g], jnp.uint32(0)))
            wt = _unpack(jnp.concatenate(wt, axis=0))
            ksk = _unpack(ks_ref[br, h, pl.ds(row0 + 64 * qb, KR // 2), :])
            s = jax.lax.dot_general(ksk, wt, NT, preferred_element_type=F32)
            if first and qb < 2:
                jfull = jax.lax.broadcasted_iota(jnp.int32, (KR, 128), 0)
                gfull = jax.lax.broadcasted_iota(jnp.int32, (KR, 128), 1) // 32
                s = jnp.where(jfull + 32 * gfull + QB * qb >= WIN, s, NEG)
            s = jnp.concatenate([jnp.where(diag_ok, s[WIN:KR], s[0:32]), s[32:WIN]], axis=0)
            st["m"][br, qb, h] = jnp.max(s, axis=0, keepdims=True)
            sb = st["unit"] % NSB
            st["unit"] += 1
            st["sb"][br, qb, h] = sb
            s_ref[sb] = s

        def pv(br, qb, h):
            sb = st["sb"][br, qb, h]
            m = st["m"][br, qb, h]
            pe = jnp.exp2(s_ref[sb, pl.ds(0, WIN // 2, stride=2), :] - m)
            po = jnp.exp2(s_ref[sb, pl.ds(1, WIN // 2, stride=2), :] - m)
            p = pltpu.pack_elementwise([pe, po], packed_dtype=BF16)
            zc = jnp.zeros((16, 128), U32)
            pc = [p[16 * k:16 * k + 16] for k in range(8)]
            pc = [pc[0] & fmask] + pc[1:] + [pc[0] & dmask]
            s1 = [jnp.where(m5, pc[k - 1] if k >= 1 else zc, pc[k] if k < 9 else zc) for k in range(10)]
            s2 = [jnp.where(m6, s1[k - 2] if k >= 2 else zc, s1[k] if k < 10 else zc) for k in range(12)]
            pt = _unpack(jnp.concatenate(s2, axis=0))
            vth = jnp.concatenate(
                [_unpack(vt_ref[br, tile0 + qb + t, 16 * h:16 * h + 16, :]) for t in range(3)], axis=1)
            o = jnp.dot(vth, pt, preferred_element_type=F32)
            o = o * pl.reciprocal(o[DH:DH + 1], approx=True)
            ot_ref[br, qb, 16 * h:16 * h + 16, :] = _pack(o)

        def outp(br, qb):
            r = jnp.dot(wot_ref[br], _unpack(ot_ref[br, qb]), preferred_element_type=F32).astype(BF16)
            rows = slice(QB * qb, QB * qb + QB)
            if br == 0:
                o_ref[rows, 0:384] = r[0:384].T
                st["ot"][qb] = r[384:448]
            else:
                r = jnp.concatenate([st["ot"][qb], r], axis=0)
                o_ref[rows, 384:896] = r.T

        need = {0: [0, 3, 4], 1: [1, 5], 2: [2, 6], 3: []}
        groups = [(br, a, qb) for br in range(2) for a in range(4) for qb in range(NQ)]
        NGR = len(groups)
        fillers = {k: [] for k in range(-1, NGR + LAG + 1)}
        def qk_tasks(br, a):
            return [functools.partial(proj_qk, br, t) for t in need[a]] + [functools.partial(build, br, a)]
        V = lambda br, t: functools.partial(proj_v, br, t)
        if ORDER == "a":
            fillers[-1] = [V(0, 0)] + qk_tasks(0, 0) + [V(0, t) for t in range(1, NQ)] + qk_tasks(0, 1)
            seq = qk_tasks(0, 2) + qk_tasks(0, 3) + qk_tasks(1, 0) + [V(1, t) for t in range(NQ)] \
                + qk_tasks(1, 1) + qk_tasks(1, 2) + qk_tasks(1, 3)
            half = NGR // 2
            pos = {}
            lst = [(qk_tasks(0, 2), 0), (qk_tasks(0, 3), 1), (qk_tasks(1, 0)[:2], 2), (qk_tasks(1, 0)[2:], 3),
                   ([V(1, t) for t in range(NQ)][:NQ // 2], 4), ([V(1, t) for t in range(NQ)][NQ // 2:], 5),
                   (qk_tasks(1, 1), 6), (qk_tasks(1, 2), 7), (qk_tasks(1, 3), 8)]
            scale = NQ // 2
            for tasks, k in lst:
                fillers[k * scale] += tasks
            for qb in range(NQ):
                fillers[half + LAG + 2 + 2 * qb].append(functools.partial(outp, 0, qb))
        for f in fillers[-1]:
            f()
        for k in range(NGR + LAG):
            if k < NGR:
                br, a, qb = groups[k]
                for b in range(4):
                    scores(br, qb, 4 * a + b)
            if k >= LAG:
                br, a, qb = groups[k - LAG]
                for b in range(4):
                    pv(br, qb, 4 * a + b)
            for f in fillers[k]:
                f()
        for qb in range(NQ):
            outp(1, qb)

    @pl.when(i == 0)
    def _():
        prep()
        body(True)

    @pl.when(i > 0)
    def _():
        body(False)


@jax.jit
def pallas_concat_heads__sliding_block__sliding_block__prompt_kernel(A_x, A_wqkv, A_wo, B_x, B_wqkv, B_wo):
    xs = pl.BlockSpec((None, D, T), lambda i: (0, 0, i))
    ws = pl.BlockSpec((D, 3 * D), lambda i: (0, 0))
    wos = pl.BlockSpec((D, D), lambda i: (0, 0))
    return pl.pallas_call(
        _kernel,
        grid=(S // T,),
        in_specs=[xs, ws, wos, xs, ws, wos],
        out_specs=pl.BlockSpec((None, T, 2 * D), lambda i: (0, i, 0)),
        out_shape=jax.ShapeDtypeStruct((1, S, 2 * D), BF16),
        scratch_shapes=[
            pltpu.VMEM((2, 512, D), BF16),
            pltpu.VMEM((2, D, 512), BF16),
            pltpu.VMEM((2, H, (HIST + S) // 2, 128), U32),
            pltpu.VMEM((2, 4, 48, 128), U32),
            pltpu.VMEM((2, S // 128 + 2, 256, 128), U32),
            pltpu.VMEM((2, NQ, 256, 128), U32),
            pltpu.VMEM((NSB, WIN, 128), F32),
        ],
        compiler_params=pltpu.CompilerParams(
            dimension_semantics=("arbitrary",),
            vmem_limit_bytes=100 * 1024 * 1024),
    )(jnp.swapaxes(A_x, 1, 2), A_wqkv, A_wo, jnp.swapaxes(B_x, 1, 2), B_wqkv, B_wo)
```

```python
import functools
import math

import jax
import jax.numpy as jnp
import jax.experimental.pallas as pl
import jax.experimental.pallas.tpu as pltpu

S = 2048
D = 448
H = 16
DH = 28
WIN = 256
T = 256
NB = S // T
QB = 128
NQ = T // QB
UNR = 2
NEG = -1e30
F32 = jnp.float32
BF16 = jnp.bfloat16
U32 = jnp.uint32
NT = (((1,), (1,)), ((), ()))
P = functools.partial

FIRST = (
    "W0 T00 W1 q000 q001 q002 W2 q003 r000 r001 q004 k000 r002 r003 q006 k003 s0000 s0010 s0003 s0013 "
    "W3 q005 V0 T01 k001 k002 v000 s0001 p0000 s0011 p0003 v001 s0002 p0001 s0012 p0010 q016 k013 p0002 "
    "q015 k012 p0013 q014 k011 q013 k010 p0011 q010 r010 q012 r013 p0012 q011 r012 r011 s0100 s0101 v010 "
    "W4 v011 O0 T10 s0102 o000 p0100 q106 k103 p0101 q105 k102 V1 s0103 p0102 o001 s0110 p0103 q104 k101 "
    "s0111 p0110 q103 k100 q102 r103 s0112 p0111 q101 r102 q100 r101 r100 v100 p0112 v101 "
    "T11 O1 s1000 s1001 q116 k113 s1002 p1000 s1003 p1001 q115 k112 s1010 p1002 p1003 v110 s1011 p1010 "
    "q114 k111 s1012 p1011 o100 s1013 p1012 q113 k110 q112 r113 p1013 q111 r112 o101 q110 r111 r110 s0113 v111")


def _pack(x):
    return pltpu.bitcast(x.astype(BF16), U32)


def _unpack(x):
    return pltpu.bitcast(x, BF16)


def _dot(a, b):
    return jnp.dot(a, b, preferred_element_type=F32)


def _kernel(xa_hbm, wa_hbm, woa_hbm, xb_hbm, wb_hbm, wob_hbm, o_hbm,
            x_v, w_v, wo_v, wvt_ref, wot_ref, wos_ref, kra_ref, krb_ref, rq_ref,
            vta_ref, vtb_ref, ot_ref, s_ref, o_v, isem, osem):
    x_hbm = (xa_hbm, xb_hbm)
    w_hbm = (wa_hbm, wb_hbm)
    wo_hbm = (woa_hbm, wob_hbm)
    kr_ref = (kra_ref, krb_ref)
    vt_ref = (vta_ref, vtb_ref)

    def rows(j, n, off, size):
        if isinstance(j, int):
            return pl.ds(j * n + off, size)
        return pl.ds(pl.multiple_of(j * n, n) + off, size)

    def x_copy(br, j, k):
        return pltpu.make_async_copy(x_hbm[br].at[0, :, pl.ds(j * T, T)], x_v.at[br, j], isem.at[k])

    def w_copy(lo, n, k):
        return pltpu.make_async_copy(w_hbm[0].at[:, pl.ds(lo, n)], w_v.at[0, :, pl.ds(lo, n)], isem.at[k])

    def o_copy(j):
        return pltpu.make_async_copy(o_v.at[j], o_hbm.at[0, rows(j, T, 0, T), :], osem.at[0])

    def o_part(r0, nr, c0, nc):
        j = NB - 1
        return pltpu.make_async_copy(o_v.at[j, pl.ds(r0, nr), pl.ds(c0, nc)],
                                     o_hbm.at[0, pl.ds(j * T + r0, nr), pl.ds(c0, nc)], osem.at[0])

    stages = [
        [x_copy(0, 0, 0)],
        [w_copy(0, 384, 1)],
        [w_copy(384, 512, 2)],
        [w_copy(2 * D, D, 3), x_copy(0, 1, 3)],
        [x_copy(1, 0, 4), pltpu.make_async_copy(w_hbm[1], w_v.at[1], isem.at[4]),
         pltpu.make_async_copy(wo_hbm[0], wo_v.at[0], isem.at[4]),
         pltpu.make_async_copy(wo_hbm[1], wo_v.at[1], isem.at[4]), x_copy(1, 1, 4)],
        [x_copy(br, jj, 5) for jj in range(2, NB) for br in range(2)],
    ]
    for stage in stages:
        for cp in stage:
            cp.start()

    def wait_stage(k):
        for cp in stages[k]:
            cp.wait()

    qscale = (DH ** -0.5) * math.log2(math.e)

    def state():
        lane = jax.lax.broadcasted_iota(jnp.int32, (1, 128), 1)
        sub = jax.lax.broadcasted_iota(jnp.int32, (8, 128), 0)
        lane8 = jax.lax.broadcasted_iota(jnp.int32, (8, 128), 1)
        return dict(
            lane=lane, lo4=sub < 4, dq=lane8 - sub,
            dr=[jnp.where((lane8 >> 5) == r, (lane8 & 31) - sub, -1) for r in range(4)],
            one04=jnp.where((sub & 3) == 0, 1.0, 0.0).astype(F32),
            x={}, tiles={}, part=[])

    def prep_v(br):
        wvt_ref[br] = pltpu.bitcast(w_v[br, :, 2 * D:3 * D].T, U32)

    def prep_o(br):
        wot_ref[br] = pltpu.bitcast(wo_v[br].T, U32)

    def proj_qk(st, br, j, t):
        if br not in st["x"]:
            st["x"][br] = x_v[br, j].T
        tl = _dot(st["x"][br], w_v[br, :, 128 * t:128 * t + 128])
        if t < 3:
            tl = tl * qscale
        elif t == 3:
            tl = tl * jnp.where(st["lane"] < 64, qscale, 1.0)
        st["tiles"][br, t] = _pack(tl)

    def proj_v(st, br, j, t):
        vt = _dot(_unpack(wvt_ref[br]), x_v[br, j, :, 128 * t:128 * t + 128])
        out = []
        for k in range(H // 2):
            r = 2 * DH * k
            mid = vt[r + 24:r + 32]
            out += [vt[r:r + 24], jnp.where(st["lo4"], mid, st["one04"]),
                    vt[r + 32:r + 56], jnp.where(st["lo4"], st["one04"], mid)]
        vt_ref[br][NQ * j + t] = _pack(jnp.concatenate(out, axis=0))

    def group_cols(st, br, col):
        t, p = divmod(col, 128)
        if p + 4 * DH <= 128:
            return st["tiles"][br, t]
        return jnp.where(st["lane"] >= p, st["tiles"][br, t], st["tiles"][br, t + 1])

    def head_lane(st, h):
        return (st["lane"] - (D + DH * h) % 128) & 127

    def build_q(st, br, j, a):
        vq = group_cols(st, br, 4 * DH * a)
        for ch in range(T // 32):
            sh = (D + 32 * (ch % 4)) % 128
            b16 = vq[16 * ch:16 * ch + 16]
            rq_ref[br, a, 16 * ch:16 * ch + 16, :] = b16 if sh == 0 else pltpu.roll(b16, sh, 1)

    def build_k(st, br, j, a):
        vk = group_cols(st, br, D + 4 * DH * a)
        z = [vk] + [pltpu.roll(vk, 32 * g, 1) for g in range(1, 4)]
        for h in range(4 * a, 4 * a + 4):
            lp = head_lane(st, h)
            k5 = (lp & 32) != 0
            k6 = (lp & 64) != 0
            kr_ref[br][h, rows(j, T // 2, 0, T // 2), :] = jnp.where(
                k6, jnp.where(k5, z[3], z[2]), jnp.where(k5, z[1], z[0]))

    def ntiles(j, qb):
        return qb + 1 if (isinstance(j, int) and j == 0) else 3

    def scores(st, br, j, qb, h):
        lp = head_lane(st, h)
        wt = []
        for g in range(4):
            r0 = 64 * qb + 16 * g
            wt.append(jnp.where((lp >= 32 * g) & (lp < 32 * g + DH), rq_ref[br, h // 4, r0:r0 + 16, :],
                                jnp.uint32(0)))
        wt = _unpack(jnp.concatenate(wt, axis=0))
        nt = ntiles(j, qb)
        kc = lambda ch, n=1: kr_ref[br][h, rows(j, T // 2, 64 * qb - 128 + 16 * ch, 16 * n), :]
        if nt == 3:
            le = [lp < 32 * (r + 1) for r in range(3)]
            dg = [kc(8 + r) for r in range(4)]
            lhs = [jnp.where(le[1], jnp.where(le[0], dg[0], dg[1]), jnp.where(le[2], dg[2], dg[3]))]
            lhs += [jnp.where(le[r], kc(r), dg[r]) for r in range(3)] + [kc(3, 5)]
        else:
            lhs = [kc(8, 4)] + ([kc(4, 4)] if nt == 2 else [])
        lhs = lhs[0] if len(lhs) == 1 else jnp.concatenate(lhs, axis=0)
        s = jax.lax.dot_general(_unpack(lhs), wt, NT, preferred_element_type=F32)
        if nt == 3:
            top = [jnp.where(st["dr"][r] >= 8 * i, s[8 * i:8 * i + 8], s[32 * r + 8 * i + 32:32 * r + 8 * i + 40])
                   for r in range(4) for i in range(4)]
            s = jnp.concatenate(top + [s[160:]], axis=0)
        else:
            top = [jnp.where(st["dq"] >= 8 * i, s[8 * i:8 * i + 8], NEG) for i in range(16)]
            s = jnp.concatenate(top + ([s[128:]] if nt == 2 else []), axis=0)
        sb = H * qb + h
        s_ref[sb, 0:s.shape[0], :] = s
        s_ref[sb, WIN:WIN + 1, :] = jnp.max(s, axis=0, keepdims=True)

    def pv(st, br, j, qb, h):
        nt = ntiles(j, qb)
        sb = H * qb + h
        e = jnp.exp2(s_ref[sb, 0:128 * min(nt, 2), :] - s_ref[sb, WIN:WIN + 1, :])
        vt = lambda t: _unpack(vt_ref[br][NQ * j + qb - 2 + t, 16 * h:16 * h + 16, :])
        if nt == 3:
            dg = [jnp.where(st["dq"] >= 8 * i, e[8 * i:8 * i + 8], 0.0) for i in range(16)]
            fr = [jnp.where(st["dq"] >= 8 * i, 0.0, e[8 * i:8 * i + 8]) for i in range(16)]
            e = jnp.concatenate([e[128:]] + dg + fr, axis=0)
            v = jnp.concatenate([vt(1), vt(2), vt(0)], axis=1)
        else:
            v = vt(2) if nt == 1 else jnp.concatenate([vt(2), vt(1)], axis=1)
        o = _dot(v, e.astype(BF16))
        lrow = 28 if h % 2 == 0 else 24
        l = o[lrow:lrow + 1]
        r = pl.reciprocal(l, approx=True)
        return o * (r * (2.0 - l * r))

    def scores4(st, br, j, qb, a):
        for h in range(4 * a, 4 * a + 4):
            scores(st, br, j, qb, h)

    def pv4(st, br, j, qb, a):
        o = [pv(st, br, j, qb, h) for h in range(4 * a, 4 * a + 4)]
        out = []
        for e, d in ((o[0], o[1]), (o[2], o[3])):
            out += [e[0:24], jnp.where(st["lo4"], e[24:32], d[24:32]), d[0:24]]
        out = jnp.concatenate(out, axis=0)
        if isinstance(j, int) and (br, j, qb) == (1, NB - 1, NQ - 1):
            o_v[NB, 0:4 * DH, 128 * a:128 * a + 128] = out.astype(BF16)
        else:
            ot_ref[br, qb, 2 * DH * a:2 * DH * (a + 1), :] = _pack(out)

    def outp(st, br, j, qb):
        r = _dot(_unpack(wot_ref[br]), _unpack(ot_ref[br, qb]))
        z = jnp.zeros((64, QB), F32)
        r = jnp.concatenate([r, z] if br == 0 else [z, r], axis=0).astype(BF16).T
        if br == 0:
            o_v[j, QB * qb:QB * (qb + 1), 0:D] = r[:, 0:D]
        else:
            o_v[j, QB * qb:QB * (qb + 1), D:2 * D] = r[:, 64:]

    def outp_part(st, a):
        r = _dot(o_v[NB, 0:4 * DH, 128 * a:128 * a + 128].T, _unpack(wos_ref[2 * DH * a:2 * DH * (a + 1), :]))
        st["part"] = [r + st["part"][0] if st["part"] else r]

    def groups(br, j):
        return [(br, j, qb, a) for qb in range(NQ) for a in range(4)]

    def half(st, br, j, pending, nxt, prv):
        q, bq, bk, v = (lambda t, f=f: P(f, st, *nxt, t) for f in (proj_qk, build_q, build_k, proj_v))
        fillers = [[q(6), bk(3)], [P(outp, st, *prv, 1)], [q(5), bk(2), q(4)], [bk(1), q(3), bk(0)],
                   [q(2), bq(3), q(1), bq(2)], [q(0), bq(1), bq(0)], [v(0)], [v(1)]]
        outp(st, *prv, 0)
        for g, fs in zip(groups(br, j), fillers):
            scores4(st, *g)
            pv4(st, *pending)
            pending = g
            for f in fs:
                f()
        return pending

    st = state()
    for tok in FIRST.split():
        op, a = tok[0], [int(ch) for ch in tok[1:]]
        if op == "W":
            wait_stage(a[0])
        elif op == "T":
            st["x"][a[0]] = x_v[a[0], a[1]].T
        elif op == "V":
            prep_v(a[0])
        elif op == "O":
            prep_o(a[0])
        else:
            dict(q=proj_qk, k=build_k, r=build_q, v=proj_v, s=scores4, p=pv4, o=outp)[op](st, *a)
    o_copy(0).start()
    wait_stage(5)

    def loop_body(it, carry):
        st = state()
        for u in range(UNR):
            j = 1 + UNR * it + u
            st["x"] = {}
            pend = half(st, 1, j, (0, j, NQ - 1, 3), (0, j + 1), (0, j))
            half(st, 0, j + 1, pend, (1, j + 1), (1, j))
            o_copy(j).start()
        return carry

    jax.lax.fori_loop(0, (NB - 2) // UNR, loop_body, 0)

    j = NB - 1
    st = state()
    wos_ref[...] = jnp.concatenate([jnp.zeros((D // 2, 64), U32), pltpu.bitcast(wo_v[1], U32)], axis=1)
    parts = [o_part(0, QB, 0, 2 * D), o_part(QB, QB, 0, 384), o_part(QB, QB, 384, 512)]
    g = [(0, j, NQ - 1, 3)] + groups(1, j)
    s4 = [P(scores4, st, *x) for x in g]
    p4 = [P(pv4, st, *x) for x in g]
    t4 = [P(outp_part, st, a) for a in range(4)]
    for f in [P(outp, st, 0, j, 0), s4[1], p4[0], s4[2], p4[1], s4[3], p4[2], P(outp, st, 0, j, 1), parts[1].start,
              s4[4], p4[3], s4[5], p4[4], s4[6], p4[5], P(outp, st, 1, j, 0), s4[7], p4[6], parts[0].start,
              s4[8], p4[7], t4[0], p4[8], t4[1], t4[2], t4[3]]:
        f()
    o_v[j, QB:2 * QB, D:2 * D] = st["part"][0][:, 64:].astype(BF16)
    parts[2].start()
    for jj in range(NB - 1):
        o_copy(jj).wait()
    for cp in parts:
        cp.wait()


@jax.jit
def pallas_concat_heads__sliding_block__sliding_block__prompt_kernel(
    A_x: jax.Array,
    A_wqkv: jax.Array,
    A_wo: jax.Array,
    B_x: jax.Array,
    B_wqkv: jax.Array,
    B_wo: jax.Array,
):
    hbm = pl.BlockSpec(memory_space=pl.ANY)
    return pl.pallas_call(
        _kernel,
        in_specs=[hbm] * 6,
        out_specs=hbm,
        out_shape=jax.ShapeDtypeStruct((1, S, 2 * D), BF16),
        scratch_shapes=[
            pltpu.VMEM((2, NB, D, T), BF16),
            pltpu.VMEM((2, D, 3 * D), BF16),
            pltpu.VMEM((2, D, D), BF16),
            pltpu.VMEM((2, D // 2, D), U32),
            pltpu.VMEM((2, D // 2, D), U32),
            pltpu.VMEM((D // 2, 512), U32),
            pltpu.VMEM((H, S // 2, 128), U32),
            pltpu.VMEM((H, S // 2, 128), U32),
            pltpu.VMEM((2, 4, T // 2, 128), U32),
            pltpu.VMEM((S // 128, 16 * H, 128), U32),
            pltpu.VMEM((S // 128, 16 * H, 128), U32),
            pltpu.VMEM((2, NQ, D // 2, 128), U32),
            pltpu.VMEM((NQ * H, WIN + 8, 128), F32),
            pltpu.VMEM((NB + 1, T, 2 * D), BF16),
            pltpu.SemaphoreType.DMA((6,)),
            pltpu.SemaphoreType.DMA((1,)),
        ],
        compiler_params=pltpu.CompilerParams(vmem_limit_bytes=100 * 1024 * 1024),
    )(jnp.swapaxes(A_x, 1, 2), A_wqkv, A_wo, jnp.swapaxes(B_x, 1, 2), B_wqkv, B_wo)
```

```python
import functools
import math

import jax
import jax.numpy as jnp
import jax.experimental.pallas as pl
import jax.experimental.pallas.tpu as pltpu

S = 2048
D = 448
H = 16
DH = 28
WIN = 256
T = 256
NB = S // T
QB = 128
NQ = T // QB
UNR = 1
NEG = -1e30
F32 = jnp.float32
BF16 = jnp.bfloat16
U32 = jnp.uint32
NT = (((1,), (1,)), ((), ()))
P = functools.partial

FIRST = (
    "W0 T00 W1 q000 q001 q002 W2 q003 r000 r001 q004 k000 r002 r003 q006 k003 s0000 s0010 s0003 s0013 "
    "W3 q005 V0 T01 k001 k002 v000 s0001 p0000 s0011 p0003 v001 s0002 p0001 s0012 p0010 q016 k013 p0002 "
    "q015 k012 p0013 q014 k011 q013 k010 p0011 q010 r010 q012 r013 p0012 q011 r012 r011 s0100 s0101 v010 "
    "W4 v011 O0 T10 s0102 o000 p0100 q106 k103 p0101 q105 k102 V1 s0103 p0102 o001 s0110 p0103 q104 k101 "
    "s0111 p0110 q103 k100 q102 r103 s0112 p0111 q101 r102 q100 r101 r100 v100 p0112 v101 "
    "T11 O1 s1000 s1001 q116 k113 s1002 p1000 s1003 p1001 q115 k112 s1010 p1002 p1003 v110 s1011 p1010 "
    "q114 k111 s1012 p1011 o100 s1013 p1012 q113 k110 q112 r113 p1013 q111 r112 o101 q110 r111 r110 s0113 v111")


def _pack(x):
    return pltpu.bitcast(x.astype(BF16), U32)


def _unpack(x):
    return pltpu.bitcast(x, BF16)


def _dot(a, b):
    return jnp.dot(a, b, preferred_element_type=F32)


def _kernel(xa_hbm, wa_hbm, woa_hbm, xb_hbm, wb_hbm, wob_hbm, o_hbm,
            x_v, w_v, wo_v, wvt_ref, wot_ref, wos_ref, kra_ref, krb_ref, rq_ref,
            vta_ref, vtb_ref, ot_ref, s_ref, o_v, isem, osem):
    x_hbm = (xa_hbm, xb_hbm)
    w_hbm = (wa_hbm, wb_hbm)
    wo_hbm = (woa_hbm, wob_hbm)
    kr_ref = (kra_ref, krb_ref)
    vt_ref = (vta_ref, vtb_ref)

    def rows(j, n, off, size):
        if isinstance(j, int):
            return pl.ds(j * n + off, size)
        return pl.ds(pl.multiple_of(j * n, n) + off, size)

    def x_copy(br, j, k):
        return pltpu.make_async_copy(x_hbm[br].at[0, :, pl.ds(j * T, T)], x_v.at[br, j], isem.at[k])

    def w_copy(lo, n, k):
        return pltpu.make_async_copy(w_hbm[0].at[:, pl.ds(lo, n)], w_v.at[0, :, pl.ds(lo, n)], isem.at[k])

    def o_copy(j):
        return pltpu.make_async_copy(o_v.at[j], o_hbm.at[0, rows(j, T, 0, T), :], osem.at[0])

    def o_part(r0, nr, c0, nc):
        j = NB - 1
        return pltpu.make_async_copy(o_v.at[j, pl.ds(r0, nr), pl.ds(c0, nc)],
                                     o_hbm.at[0, pl.ds(j * T + r0, nr), pl.ds(c0, nc)], osem.at[0])

    stages = [
        [x_copy(0, 0, 0)],
        [w_copy(0, 384, 1)],
        [w_copy(384, 512, 2)],
        [w_copy(2 * D, D, 3), x_copy(0, 1, 3)],
        [x_copy(1, 0, 4), pltpu.make_async_copy(w_hbm[1], w_v.at[1], isem.at[4]),
         pltpu.make_async_copy(wo_hbm[0], wo_v.at[0], isem.at[4]),
         pltpu.make_async_copy(wo_hbm[1], wo_v.at[1], isem.at[4]), x_copy(1, 1, 4)],
        [x_copy(br, jj, 5) for jj in range(2, NB) for br in range(2)],
    ]
    for stage in stages:
        for cp in stage:
            cp.start()

    def wait_stage(k):
        for cp in stages[k]:
            cp.wait()

    qscale = (DH ** -0.5) * math.log2(math.e)

    def state():
        lane = jax.lax.broadcasted_iota(jnp.int32, (1, 128), 1)
        sub = jax.lax.broadcasted_iota(jnp.int32, (8, 128), 0)
        key = jax.lax.broadcasted_iota(jnp.int32, (QB, QB), 0)
        qry = jax.lax.broadcasted_iota(jnp.int32, (QB, QB), 1)
        return dict(
            lane=lane, lo4=sub < 4, tri=key <= qry, tri32=jnp.where((key >> 5) == (qry >> 5), qry - key, -1) >= 0,
            one04=jnp.where((sub & 3) == 0, 1.0, 0.0).astype(F32),
            x={}, tiles={}, part=[])

    def prep_v(br):
        wvt_ref[br] = pltpu.bitcast(w_v[br, :, 2 * D:3 * D].T, U32)

    def prep_o(br):
        wot_ref[br] = pltpu.bitcast(wo_v[br].T, U32)

    def proj_qk(st, br, j, t):
        if br not in st["x"]:
            st["x"][br] = x_v[br, j].T
        tl = _dot(st["x"][br], w_v[br, :, 128 * t:128 * t + 128])
        if t < 3:
            tl = tl * qscale
        elif t == 3:
            tl = tl * jnp.where(st["lane"] < 64, qscale, 1.0)
        st["tiles"][br, t] = _pack(tl)

    def proj_v(st, br, j, t):
        vt = _dot(_unpack(wvt_ref[br]), x_v[br, j, :, 128 * t:128 * t + 128])
        out = []
        for k in range(H // 2):
            r = 2 * DH * k
            mid = vt[r + 24:r + 32]
            out += [vt[r:r + 24], jnp.where(st["lo4"], mid, st["one04"]),
                    vt[r + 32:r + 56], jnp.where(st["lo4"], st["one04"], mid)]
        vt_ref[br][NQ * j + t] = _pack(jnp.concatenate(out, axis=0))

    def group_cols(st, br, col):
        t, p = divmod(col, 128)
        if p + 4 * DH <= 128:
            return st["tiles"][br, t]
        return jnp.where(st["lane"] >= p, st["tiles"][br, t], st["tiles"][br, t + 1])

    def head_lane(st, h):
        return (st["lane"] - (D + DH * h) % 128) & 127

    def build_q(st, br, j, a):
        vq = group_cols(st, br, 4 * DH * a)
        for ch in range(T // 32):
            sh = (D + 32 * (ch % 4)) % 128
            b16 = vq[16 * ch:16 * ch + 16]
            rq_ref[br, a, 16 * ch:16 * ch + 16, :] = b16 if sh == 0 else pltpu.roll(b16, sh, 1)

    def build_k(st, br, j, a):
        vk = group_cols(st, br, D + 4 * DH * a)
        z = [vk] + [pltpu.roll(vk, 32 * g, 1) for g in range(1, 4)]
        for h in range(4 * a, 4 * a + 4):
            lp = head_lane(st, h)
            k5 = (lp & 32) != 0
            k6 = (lp & 64) != 0
            kr_ref[br][h, rows(j, T // 2, 0, T // 2), :] = jnp.where(
                k6, jnp.where(k5, z[3], z[2]), jnp.where(k5, z[1], z[0]))

    def ntiles(j, qb):
        return qb + 1 if (isinstance(j, int) and j == 0) else 3

    def scores(st, br, j, qb, h):
        lp = head_lane(st, h)
        wt = []
        for g in range(4):
            r0 = 64 * qb + 16 * g
            wt.append(jnp.where((lp >= 32 * g) & (lp < 32 * g + DH), rq_ref[br, h // 4, r0:r0 + 16, :],
                                jnp.uint32(0)))
        wt = _unpack(jnp.concatenate(wt, axis=0))
        nt = ntiles(j, qb)
        kc = lambda ch, n=1: kr_ref[br][h, rows(j, T // 2, 64 * qb - 128 + 16 * ch, 16 * n), :]
        if nt == 3:
            le = [lp < 32 * (r + 1) for r in range(3)]
            dg = [kc(8 + r) for r in range(4)]
            lhs = [jnp.where(le[1], jnp.where(le[0], dg[0], dg[1]), jnp.where(le[2], dg[2], dg[3]))]
            lhs += [jnp.where(le[r], kc(r), dg[r]) for r in range(3)] + [kc(3, 5)]
        else:
            lhs = [kc(8, 4)] + ([kc(4, 4)] if nt == 2 else [])
        lhs = lhs[0] if len(lhs) == 1 else jnp.concatenate(lhs, axis=0)
        s = jax.lax.dot_general(_unpack(lhs), wt, NT, preferred_element_type=F32)
        if nt == 3:
            top = jax.lax.select(st["tri32"], jnp.concatenate([s[0:32]] * 4, axis=0), s[32:160])
            s = jnp.concatenate([top, s[160:]], axis=0)
        else:
            top = jnp.where(st["tri"], s[0:128], NEG)
            s = top if nt == 1 else jnp.concatenate([top, s[128:]], axis=0)
        sb = H * qb + h
        s_ref[sb, 0:s.shape[0], :] = s
        s_ref[sb, WIN:WIN + 1, :] = jnp.max(s, axis=0, keepdims=True)

    def pv(st, br, j, qb, h):
        nt = ntiles(j, qb)
        sb = H * qb + h
        e = jnp.exp2(s_ref[sb, 0:128 * min(nt, 2), :] - s_ref[sb, WIN:WIN + 1, :])
        vt = lambda t: _unpack(vt_ref[br][NQ * j + qb - 2 + t, 16 * h:16 * h + 16, :])
        if nt == 3:
            top = e[0:128]
            e = jnp.concatenate([e[128:], jnp.where(st["tri"], top, 0.0), jnp.where(st["tri"], 0.0, top)], axis=0)
            v = jnp.concatenate([vt(1), vt(2), vt(0)], axis=1)
        else:
            v = vt(2) if nt == 1 else jnp.concatenate([vt(2), vt(1)], axis=1)
        o = _dot(v, e.astype(BF16))
        lrow = 28 if h % 2 == 0 else 24
        l = o[lrow:lrow + 1]
        r = pl.reciprocal(l, approx=True)
        return o * (r * (2.0 - l * r))

    def scores4(st, br, j, qb, a):
        for h in range(4 * a, 4 * a + 4):
            scores(st, br, j, qb, h)

    def pv4(st, br, j, qb, a):
        o = [pv(st, br, j, qb, h) for h in range(4 * a, 4 * a + 4)]
        out = []
        for e, d in ((o[0], o[1]), (o[2], o[3])):
            out += [e[0:24], jnp.where(st["lo4"], e[24:32], d[24:32]), d[0:24]]
        out = jnp.concatenate(out, axis=0)
        if isinstance(j, int) and (br, j, qb) == (1, NB - 1, NQ - 1):
            o_v[NB, 0:4 * DH, 128 * a:128 * a + 128] = out.astype(BF16)
        else:
            ot_ref[br, qb, 2 * DH * a:2 * DH * (a + 1), :] = _pack(out)

    def outp(st, br, j, qb):
        r = _dot(_unpack(wot_ref[br]), _unpack(ot_ref[br, qb]))
        z = jnp.zeros((64, QB), F32)
        r = jnp.concatenate([r, z] if br == 0 else [z, r], axis=0).astype(BF16).T
        if br == 0:
            o_v[j, QB * qb:QB * (qb + 1), 0:D] = r[:, 0:D]
        else:
            o_v[j, QB * qb:QB * (qb + 1), D:2 * D] = r[:, 64:]

    def outp_part(st, a):
        r = _dot(o_v[NB, 0:4 * DH, 128 * a:128 * a + 128].T, _unpack(wos_ref[2 * DH * a:2 * DH * (a + 1), :]))
        st["part"] = [r + st["part"][0] if st["part"] else r]

    def groups(br, j):
        return [(br, j, qb, a) for qb in range(NQ) for a in range(4)]

    def half(st, br, j, pending, nxt, prv):
        q, bq, bk, v = (lambda t, f=f: P(f, st, *nxt, t) for f in (proj_qk, build_q, build_k, proj_v))
        fillers = [[q(6), bk(3)], [P(outp, st, *prv, 1)], [q(5), bk(2), q(4)], [bk(1), q(3), bk(0)],
                   [q(2), bq(3), q(1), bq(2)], [q(0), bq(1), bq(0)], [v(0)], [v(1)]]
        outp(st, *prv, 0)
        for g, fs in zip(groups(br, j), fillers):
            scores4(st, *g)
            pv4(st, *pending)
            pending = g
            for f in fs:
                f()
        return pending

    st = state()
    for tok in FIRST.split():
        op, a = tok[0], [int(ch) for ch in tok[1:]]
        if op == "W":
            wait_stage(a[0])
        elif op == "T":
            st["x"][a[0]] = x_v[a[0], a[1]].T
        elif op == "V":
            prep_v(a[0])
        elif op == "O":
            prep_o(a[0])
        else:
            dict(q=proj_qk, k=build_k, r=build_q, v=proj_v, s=scores4, p=pv4, o=outp)[op](st, *a)
    o_copy(0).start()
    wait_stage(5)

    def loop_body(it, carry):
        st = state()
        for u in range(UNR):
            j = 1 + UNR * it + u
            st["x"] = {}
            pend = half(st, 1, j, (0, j, NQ - 1, 3), (0, j + 1), (0, j))
            half(st, 0, j + 1, pend, (1, j + 1), (1, j))
            o_copy(j).start()
        return carry

    jax.lax.fori_loop(0, (NB - 2) // UNR, loop_body, 0)

    j = NB - 1
    st = state()
    wos_ref[...] = jnp.concatenate([jnp.zeros((D // 2, 64), U32), pltpu.bitcast(wo_v[1], U32)], axis=1)
    parts = [o_part(0, QB, 0, 2 * D), o_part(QB, QB, 0, 384), o_part(QB, QB, 384, 512)]
    g = [(0, j, NQ - 1, 3)] + groups(1, j)
    s4 = [P(scores4, st, *x) for x in g]
    p4 = [P(pv4, st, *x) for x in g]
    t4 = [P(outp_part, st, a) for a in range(4)]
    for f in [P(outp, st, 0, j, 0), s4[1], p4[0], s4[2], p4[1], s4[3], p4[2], P(outp, st, 0, j, 1), parts[1].start,
              s4[4], p4[3], s4[5], p4[4], s4[6], p4[5], P(outp, st, 1, j, 0), s4[7], p4[6], parts[0].start,
              s4[8], p4[7], t4[0], p4[8], t4[1], t4[2], t4[3]]:
        f()
    o_v[j, QB:2 * QB, D:2 * D] = st["part"][0][:, 64:].astype(BF16)
    parts[2].start()
    for jj in range(NB - 1):
        o_copy(jj).wait()
    for cp in parts:
        cp.wait()


@jax.jit
def pallas_concat_heads__sliding_block__sliding_block__prompt_kernel(
    A_x: jax.Array,
    A_wqkv: jax.Array,
    A_wo: jax.Array,
    B_x: jax.Array,
    B_wqkv: jax.Array,
    B_wo: jax.Array,
):
    hbm = pl.BlockSpec(memory_space=pl.ANY)
    return pl.pallas_call(
        _kernel,
        in_specs=[hbm] * 6,
        out_specs=hbm,
        out_shape=jax.ShapeDtypeStruct((1, S, 2 * D), BF16),
        scratch_shapes=[
            pltpu.VMEM((2, NB, D, T), BF16),
            pltpu.VMEM((2, D, 3 * D), BF16),
            pltpu.VMEM((2, D, D), BF16),
            pltpu.VMEM((2, D // 2, D), U32),
            pltpu.VMEM((2, D // 2, D), U32),
            pltpu.VMEM((D // 2, 512), U32),
            pltpu.VMEM((H, S // 2, 128), U32),
            pltpu.VMEM((H, S // 2, 128), U32),
            pltpu.VMEM((2, 4, T // 2, 128), U32),
            pltpu.VMEM((S // 128, 16 * H, 128), U32),
            pltpu.VMEM((S // 128, 16 * H, 128), U32),
            pltpu.VMEM((2, NQ, D // 2, 128), U32),
            pltpu.VMEM((NQ * H, WIN + 8, 128), F32),
            pltpu.VMEM((NB + 1, T, 2 * D), BF16),
            pltpu.SemaphoreType.DMA((6,)),
            pltpu.SemaphoreType.DMA((1,)),
        ],
        compiler_params=pltpu.CompilerParams(vmem_limit_bytes=100 * 1024 * 1024),
    )(jnp.swapaxes(A_x, 1, 2), A_wqkv, A_wo, jnp.swapaxes(B_x, 1, 2), B_wqkv, B_wo)
```

```python
import functools
import math

import jax
import jax.numpy as jnp
import jax.experimental.pallas as pl
import jax.experimental.pallas.tpu as pltpu

S = 2048
D = 448
H = 16
DH = 28
WIN = 256
T = 256
NB = S // T
QB = 128
NQ = T // QB
UNR = 3
NEG = -1e30
F32 = jnp.float32
BF16 = jnp.bfloat16
U32 = jnp.uint32
NT = (((1,), (1,)), ((), ()))
P = functools.partial

FIRST = (
    "W0 T00 W1 q000 q001 q002 W2 q003 r000 r001 q004 k000 r002 r003 q006 k003 s0000 s0010 s0003 s0013 W3 "
    "q005 V0 T01 k002 v000 k001 s0001 p0000 s0011 p0003 s0002 p0001 s0012 v001 q013 p0010 q014 k010 p0002 "
    "q015 k011 p0013 p0011 q010 r010 q016 k012 q011 r011 p0012 k013 q012 r012 r013 s0100 s0101 v010 W4 "
    "v011 O0 s0102 o000 p0100 T10 s0103 q106 V1 k103 p0101 q105 k102 p0102 p0103 o001 s0110 q104 s0111 "
    "p0110 q103 k100 k101 s0112 q102 r103 p0111 q101 q100 r101 r100 r102 O1 p0112 v100 v101 T11 s1000 "
    "s1001 q116 k113 s1002 p1000 s1003 p1001 q115 k112 s1010 p1003 p1002 q114 s1011 s1012 v110 k111 o100 "
    "p1010 p1011 q112 s1013 q113 r113 k110 p1012 p1013 q111 r112 q110 o101 r111 r110 s0113 v111 ")


def _pack(x):
    return pltpu.bitcast(x.astype(BF16), U32)


def _unpack(x):
    return pltpu.bitcast(x, BF16)


def _dot(a, b):
    return jnp.dot(a, b, preferred_element_type=F32)


def _body(xa_hbm, wa_hbm, woa_hbm, xb_hbm, wb_hbm, wob_hbm, o_hbm,
          x_v, w_v, wo_v, xt_ref, tl_ref, wvt_ref, wot_ref, wos_ref, kra_ref, krb_ref, rq_ref,
          vta_ref, vtb_ref, ot_ref, s_ref, o_v, isem, osem):
    x_hbm = (xa_hbm, xb_hbm)
    w_hbm = (wa_hbm, wb_hbm)
    wo_hbm = (woa_hbm, wob_hbm)
    kr_ref = (kra_ref, krb_ref)
    vt_ref = (vta_ref, vtb_ref)

    def rows(j, n, off, size):
        if isinstance(j, int):
            return pl.ds(j * n + off, size)
        return pl.ds(pl.multiple_of(j * n, n) + off, size)

    def x_copy(br, j, k):
        return pltpu.make_async_copy(x_hbm[br].at[0, :, pl.ds(j * T, T)], x_v.at[br, j], isem.at[k])

    def w_copy(lo, n, k):
        return pltpu.make_async_copy(w_hbm[0].at[:, pl.ds(lo, n)], w_v.at[0, :, pl.ds(lo, n)], isem.at[k])

    def o_copy(j, n):
        return pltpu.make_async_copy(o_v.at[rows(j, T, 0, n * T), :], o_hbm.at[0, rows(j, T, 0, n * T), :], osem.at[0])

    def o_part(r0, nr, c0, nc):
        j = NB - 1
        return pltpu.make_async_copy(o_v.at[pl.ds(j * T + r0, nr), pl.ds(c0, nc)],
                                     o_hbm.at[0, pl.ds(j * T + r0, nr), pl.ds(c0, nc)], osem.at[0])

    stages = [
        [x_copy(0, 0, 0)],
        [w_copy(0, 384, 1)],
        [w_copy(384, 256, 2), w_copy(768, 128, 2)],
        [w_copy(640, 128, 3), w_copy(2 * D, D, 3), x_copy(0, 1, 3)],
        [x_copy(1, 0, 4), pltpu.make_async_copy(w_hbm[1], w_v.at[1], isem.at[4]),
         pltpu.make_async_copy(wo_hbm[0], wo_v.at[0], isem.at[4]),
         pltpu.make_async_copy(wo_hbm[1], wo_v.at[1], isem.at[4]), x_copy(1, 1, 4)],
        [x_copy(br, jj, 5) for jj in range(2, NB) for br in range(2)],
    ]
    for stage in stages:
        for cp in stage:
            cp.start()

    def wait_stage(k):
        for cp in stages[k]:
            cp.wait()

    qscale = (DH ** -0.5) * math.log2(math.e)

    def state():
        lane = jax.lax.broadcasted_iota(jnp.int32, (1, 128), 1)
        sub = jax.lax.broadcasted_iota(jnp.int32, (8, 128), 0)
        key = jax.lax.broadcasted_iota(jnp.int32, (QB, QB), 0)
        qry = jax.lax.broadcasted_iota(jnp.int32, (QB, QB), 1)
        return dict(
            lane=lane, lo4=sub < 4, tri=key <= qry, tri32=jnp.where((key >> 5) == (qry >> 5), qry - key, -1) >= 0,
            one04=jnp.where((sub & 3) == 0, 1.0, 0.0).astype(F32),
            m={}, part=[], end=True)

    def prep_v(br):
        wvt_ref[br] = pltpu.bitcast(w_v[br, :, 2 * D:3 * D].T, U32)

    def prep_o(br):
        wot_ref[br] = pltpu.bitcast(wo_v[br].T, U32)

    def xpose(br, j):
        xt_ref[br] = pltpu.bitcast(x_v[br, j].T, U32)

    def proj_qk(st, br, j, t):
        tl = _dot(_unpack(xt_ref[br]), w_v[br, :, 128 * t:128 * t + 128])
        if t < 3:
            tl = tl * qscale
        elif t == 3:
            tl = tl * jnp.where(st["lane"] < 64, qscale, 1.0)
        tl_ref[br, t] = _pack(tl)

    def proj_v(st, br, j, t):
        vt = _dot(_unpack(wvt_ref[br]), x_v[br, j, :, 128 * t:128 * t + 128])
        out = []
        for k in range(H // 2):
            r = 2 * DH * k
            mid = vt[r + 24:r + 32]
            out += [vt[r:r + 24], jnp.where(st["lo4"], mid, st["one04"]),
                    vt[r + 32:r + 56], jnp.where(st["lo4"], st["one04"], mid)]
        vt_ref[br][NQ * j + t] = _pack(jnp.concatenate(out, axis=0))

    def group_cols(st, br, col):
        t, p = divmod(col, 128)
        if p + 4 * DH <= 128:
            return tl_ref[br, t]
        return jnp.where(st["lane"] >= p, tl_ref[br, t], tl_ref[br, t + 1])

    def head_lane(st, h):
        return (st["lane"] - (D + DH * h) % 128) & 127

    def build_q(st, br, j, a):
        vq = group_cols(st, br, 4 * DH * a)
        for ch in range(T // 32):
            sh = (D + 32 * (ch % 4)) % 128
            b16 = vq[16 * ch:16 * ch + 16]
            rq_ref[br, a, 16 * ch:16 * ch + 16, :] = b16 if sh == 0 else pltpu.roll(b16, sh, 1)

    def build_k(st, br, j, a):
        vk = group_cols(st, br, D + 4 * DH * a)
        z = [vk] + [pltpu.roll(vk, 32 * g, 1) for g in range(1, 4)]
        for h in range(4 * a, 4 * a + 4):
            lp = head_lane(st, h)
            k5 = (lp & 32) != 0
            k6 = (lp & 64) != 0
            kr_ref[br][h, rows(j, T // 2, 0, T // 2), :] = jnp.where(
                k6, jnp.where(k5, z[3], z[2]), jnp.where(k5, z[1], z[0]))

    def ntiles(j, qb):
        return qb + 1 if (isinstance(j, int) and j == 0) else 3

    def carried(br, j, qb, h):
        return br == 0 and qb == NQ - 1 and h >= H - 4 and ntiles(j, qb) == 3

    def scores(st, br, j, qb, h):
        lp = head_lane(st, h)
        wt = []
        for g in range(4):
            r0 = 64 * qb + 16 * g
            wt.append(jnp.where((lp >= 32 * g) & (lp < 32 * g + DH), rq_ref[br, h // 4, r0:r0 + 16, :],
                                jnp.uint32(0)))
        wt = _unpack(jnp.concatenate(wt, axis=0))
        nt = ntiles(j, qb)
        kc = lambda ch, n=1: kr_ref[br][h, rows(j, T // 2, 64 * qb - 128 + 16 * ch, 16 * n), :]
        if nt == 3:
            le = [lp < 32 * (r + 1) for r in range(3)]
            dg = [kc(8 + r) for r in range(4)]
            lhs = jnp.concatenate(
                [kc(4, 4), jnp.where(le[1], jnp.where(le[0], dg[0], dg[1]), jnp.where(le[2], dg[2], dg[3]))]
                + [jnp.where(le[r], kc(r), dg[r]) for r in range(3)] + [kc(3)], axis=0)
        else:
            lhs = kc(12 - 4 * nt, 4 * nt)
        s = jax.lax.dot_general(_unpack(lhs), wt, NT, preferred_element_type=F32)
        if nt == 3:
            edge = jax.lax.select(st["tri32"], jnp.concatenate([s[128:160]] * 4, axis=0), s[160:])
        else:
            edge = jnp.where(st["tri"], s[128 * (nt - 1):], NEG)
        s = edge if nt == 1 else jnp.concatenate([s[0:128], edge], axis=0)
        sb = H * qb + h
        s_ref[sb, 0:s.shape[0], :] = s
        m = jnp.max(s, axis=0, keepdims=True)
        if carried(br, j, qb, h) and st["end"]:
            s_ref[sb, WIN:WIN + 1, :] = m
        else:
            st["m"][sb] = m

    def pv(st, br, j, qb, h):
        nt = ntiles(j, qb)
        sb = H * qb + h
        m = st["m"].pop(sb) if sb in st["m"] else s_ref[sb, WIN:WIN + 1, :]
        e = jnp.exp2(s_ref[sb, 0:128 * min(nt, 2), :] - m)
        vt = lambda t: _unpack(vt_ref[br][NQ * j + qb - 2 + t, 16 * h:16 * h + 16, :])
        if nt == 3:
            edge = e[128:]
            e = jnp.concatenate([jnp.where(st["tri"], edge, 0.0), jnp.where(st["tri"], 0.0, edge), e[0:128]], axis=0)
            v = jnp.concatenate([vt(2), vt(0), vt(1)], axis=1)
        else:
            v = vt(2) if nt == 1 else jnp.concatenate([vt(1), vt(2)], axis=1)
        o = _dot(v, e.astype(BF16))
        lrow = 28 if h % 2 == 0 else 24
        l = o[lrow:lrow + 1]
        r = pl.reciprocal(l, approx=True)
        return o * (r * (2.0 - l * r))

    def scores4(st, br, j, qb, a):
        for h in range(4 * a, 4 * a + 4):
            scores(st, br, j, qb, h)

    def pv4(st, br, j, qb, a):
        o = [pv(st, br, j, qb, h) for h in range(4 * a, 4 * a + 4)]
        out = []
        for e, d in ((o[0], o[1]), (o[2], o[3])):
            out += [e[0:24], jnp.where(st["lo4"], e[24:32], d[24:32]), d[0:24]]
        out = jnp.concatenate(out, axis=0)
        if isinstance(j, int) and (br, j, qb) == (1, NB - 1, NQ - 1):
            o_v[S:S + 4 * DH, 128 * a:128 * a + 128] = out.astype(BF16)
        else:
            ot_ref[br, qb, 2 * DH * a:2 * DH * (a + 1), :] = _pack(out)

    def outp(st, br, j, qb):
        r = _dot(_unpack(wot_ref[br]), _unpack(ot_ref[br, qb]))
        z = jnp.zeros((64, QB), F32)
        r = jnp.concatenate([r, z] if br == 0 else [z, r], axis=0).astype(BF16).T
        if br == 0:
            o_v[rows(j, T, QB * qb, QB), 0:D] = r[:, 0:D]
        else:
            o_v[rows(j, T, QB * qb, QB), D:2 * D] = r[:, 64:]

    def outp_part(st, a):
        r = _dot(o_v[S:S + 4 * DH, 128 * a:128 * a + 128].T, _unpack(wos_ref[2 * DH * a:2 * DH * (a + 1), :]))
        st["part"] = [r + st["part"][0] if st["part"] else r]

    def groups(br, j):
        return [(br, j, qb, a) for qb in range(NQ) for a in range(4)]

    def half(st, br, j, pending, nxt, prv):
        q, bq, bk, v = (lambda t, f=f: P(f, st, *nxt, t) for f in (proj_qk, build_q, build_k, proj_v))
        fillers = [[P(xpose, *nxt), q(6), bk(3)], [P(outp, st, *prv, 1)], [q(5), bk(2), q(4)], [bk(1), q(3), bk(0)],
                   [q(2), bq(3), q(1), bq(2)], [q(0), bq(1), bq(0)], [v(0)], [v(1)]]
        outp(st, *prv, 0)
        for g, fs in zip(groups(br, j), fillers):
            scores4(st, *g)
            pv4(st, *pending)
            pending = g
            for f in fs:
                f()
        return pending

    st = state()
    for tok in FIRST.split():
        op, a = tok[0], [int(ch) for ch in tok[1:]]
        if op == "W":
            wait_stage(a[0])
        elif op == "T":
            xpose(*a)
        elif op == "V":
            prep_v(a[0])
        elif op == "O":
            prep_o(a[0])
        else:
            dict(q=proj_qk, k=build_k, r=build_q, v=proj_v, s=scores4, p=pv4, o=outp)[op](st, *a)
    o_copy(0, 1).start()
    wait_stage(5)

    def loop_body(it, carry):
        st = state()
        for u in range(UNR):
            j = 1 + UNR * it + u
            st["end"] = u == UNR - 1
            pend = half(st, 1, j, (0, j, NQ - 1, 3), (0, j + 1), (0, j))
            half(st, 0, j + 1, pend, (1, j + 1), (1, j))
        o_copy(1 + UNR * it, UNR).start()
        return carry

    jax.lax.fori_loop(0, (NB - 2) // UNR, loop_body, 0)

    j = NB - 1
    st = state()
    wos_ref[...] = jnp.concatenate([jnp.zeros((D // 2, 64), U32), pltpu.bitcast(wo_v[1], U32)], axis=1)
    parts = [o_part(0, QB, 0, 2 * D), o_part(QB, QB, 0, 384)] + [o_part(QB + 32 * k, 32, 384, 512) for k in range(4)]
    g = [(0, j, NQ - 1, 3)] + groups(1, j)
    s4 = [P(scores4, st, *x) for x in g]
    p4 = [P(pv4, st, *x) for x in g]
    t4 = [P(outp_part, st, a) for a in range(4)]
    for f in [P(outp, st, 0, j, 0), s4[1], p4[0], s4[2], p4[1], s4[3], p4[2], P(outp, st, 0, j, 1), parts[1].start,
              s4[4], p4[3], s4[5], p4[4], s4[6], p4[5], P(outp, st, 1, j, 0), s4[7], p4[6], parts[0].start,
              s4[8], p4[7], t4[0], p4[8], t4[1], t4[2], t4[3]]:
        f()
    for k in range(4):
        o_v[rows(j, T, QB + 32 * k, 32), D:2 * D] = st["part"][0][32 * k:32 * (k + 1), 64:].astype(BF16)
        parts[2 + k].start()
    o_copy(0, 1).wait()
    for jj in range(1, NB - 1, UNR):
        o_copy(jj, UNR).wait()
    for cp in parts:
        cp.wait()


def _kernel(*refs):
    pl.when(pl.program_id(0) == 1)(lambda: _body(*refs))


@jax.jit
def pallas_concat_heads__sliding_block__sliding_block__prompt_kernel(
    A_x: jax.Array,
    A_wqkv: jax.Array,
    A_wo: jax.Array,
    B_x: jax.Array,
    B_wqkv: jax.Array,
    B_wo: jax.Array,
):
    hbm = pl.BlockSpec(memory_space=pl.ANY)
    return pl.pallas_call(
        _kernel,
        grid=(2,),
        in_specs=[hbm] * 6,
        out_specs=hbm,
        out_shape=jax.ShapeDtypeStruct((1, S, 2 * D), BF16),
        scratch_shapes=[
            pltpu.VMEM((2, NB, D, T), BF16),
            pltpu.VMEM((2, D, 3 * D), BF16),
            pltpu.VMEM((2, D, D), BF16),
            pltpu.VMEM((2, T // 2, D), U32),
            pltpu.VMEM((2, 7, T // 2, 128), U32),
            pltpu.VMEM((2, D // 2, D), U32),
            pltpu.VMEM((2, D // 2, D), U32),
            pltpu.VMEM((D // 2, 512), U32),
            pltpu.VMEM((H, S // 2, 128), U32),
            pltpu.VMEM((H, S // 2, 128), U32),
            pltpu.VMEM((2, 4, T // 2, 128), U32),
            pltpu.VMEM((S // 128, 16 * H, 128), U32),
            pltpu.VMEM((S // 128, 16 * H, 128), U32),
            pltpu.VMEM((2, NQ, D // 2, 128), U32),
            pltpu.VMEM((NQ * H, WIN + 8, 128), F32),
            pltpu.VMEM((S + 4 * DH, 2 * D), BF16),
            pltpu.SemaphoreType.DMA((6,)),
            pltpu.SemaphoreType.DMA((1,)),
        ],
        compiler_params=pltpu.CompilerParams(
            dimension_semantics=("arbitrary",), vmem_limit_bytes=100 * 1024 * 1024),
    )(jnp.swapaxes(A_x, 1, 2), A_wqkv, A_wo, jnp.swapaxes(B_x, 1, 2), B_wqkv, B_wo)
```
